```python
import os as _os
_os.environ.setdefault("JAX_PLATFORMS", "cpu")
import jax
import jax.numpy as jnp

def _softmax(x, axis=-1):
    return jax.nn.softmax(x, axis=axis)
def _gelu(x):
    return jax.nn.gelu(x, approximate=True)
def _silu(x):
    return jax.nn.silu(x)
def _sigmoid(x):
    return jax.nn.sigmoid(x)
def _layernorm(x, axis=-1, eps=1e-5):
    m = jnp.mean(x, axis=axis, keepdims=True)
    v = jnp.var(x, axis=axis, keepdims=True)
    return (x - m) / jnp.sqrt(v + eps)
def _scatter_add(tgt, idx, src, axis=0):
    return tgt.at[idx].add(src)
def _segment_sum(src, seg, n):
    return jax.ops.segment_sum(src, seg, n)
class _Rng:
    def __init__(self, key):
        self._k = key
    def _next(self):
        self._k, sub = jax.random.split(self._k)
        return sub
    def normal(self, shape):
        return jax.random.normal(self._next(), shape, dtype=jnp.bfloat16)
    def randint(self, lo, hi, shape):
        return jax.random.randint(self._next(), shape, lo, hi, dtype=jnp.int32)
    def uniform(self, shape, lo=0.0, hi=1.0):
        return jax.random.uniform(self._next(), shape, jnp.bfloat16, lo, hi)
    def permutation(self, n):
        return jax.random.permutation(self._next(), n)


kernel_name = 'concat_heads__mha_block_cached__mha_block_cached__near_ridge'

def setup_inputs():
    _rng = _Rng(jax.random.key(int.from_bytes(__import__("os").urandom(4), "little")))
    _w = (lambda a: (lambda t: t.astype(jnp.bfloat16) if jnp.issubdtype(t.dtype, jnp.floating) else t)(jnp.asarray(a)))
    def _A_setup():
        B, Sq, D = 16, 32, 1024
        H, Sk, Dh = 32, 32, 128
        return {
            "x": _w((lambda *s: _rng.normal(s) * 0.8)(B, Sq, D)),
            "k_cache": _w((lambda *s: _rng.normal(s) * 0.8)(B, H, Sk, Dh)),
            "v_cache": _w((lambda *s: _rng.normal(s) * 0.05)(B, H, Sk, Dh)),
            "wq": _w((lambda *s: _rng.normal(s) * 0.8)(D, H * Dh) * (D ** -0.5)),
            "wo": _w((lambda *s: _rng.normal(s) * 0.05)(H * Dh, D) * ((H * Dh) ** -0.5)),
        }
    _A_in = _A_setup()

    def _B_setup():
        B, Sq, D = 16, 32, 1024
        H, Sk, Dh = 32, 32, 128
        return {
            "x": _w((lambda *s: _rng.normal(s) * 0.8)(B, Sq, D)),
            "k_cache": _w((lambda *s: _rng.normal(s) * 0.8)(B, H, Sk, Dh)),
            "v_cache": _w((lambda *s: _rng.normal(s) * 0.05)(B, H, Sk, Dh)),
            "wq": _w((lambda *s: _rng.normal(s) * 0.8)(D, H * Dh) * (D ** -0.5)),
            "wo": _w((lambda *s: _rng.normal(s) * 0.05)(H * Dh, D) * ((H * Dh) ** -0.5)),
        }
    _B_in = _B_setup()

    return {
        "A_x": _A_in["x"],
        "A_k_cache": _A_in["k_cache"],
        "A_v_cache": _A_in["v_cache"],
        "A_wq": _A_in["wq"],
        "A_wo": _A_in["wo"],
        "B_x": _B_in["x"],
        "B_k_cache": _B_in["k_cache"],
        "B_v_cache": _B_in["v_cache"],
        "B_wq": _B_in["wq"],
        "B_wo": _B_in["wo"],
    }

def reference(A_x, A_k_cache, A_v_cache, A_wq, A_wo, B_x, B_k_cache, B_v_cache, B_wq, B_wo):
    def _A_ref(x, k_cache, v_cache, wq, wo):
        B, Sq, D = x.shape
        H, Dh = 32, 128
        q = (lambda x, *d: x.transpose(*d))((x @ wq).reshape(B, Sq, H, Dh), 0, 2, 1, 3)
        scores = jnp.einsum("bhqd,bhkd->bhqk", q, k_cache) * (Dh ** -0.5)
        p = _softmax(scores, axis=-1)
        o = jnp.einsum("bhqk,bhkd->bhqd", p, v_cache)
        return (lambda x, *d: x.transpose(*d))(o, 0, 2, 1, 3).reshape(B, Sq, H * Dh) @ wo

    def _B_ref(x, k_cache, v_cache, wq, wo):
        B, Sq, D = x.shape
        H, Dh = 32, 128
        q = (lambda x, *d: x.transpose(*d))((x @ wq).reshape(B, Sq, H, Dh), 0, 2, 1, 3)
        scores = jnp.einsum("bhqd,bhkd->bhqk", q, k_cache) * (Dh ** -0.5)
        p = _softmax(scores, axis=-1)
        o = jnp.einsum("bhqk,bhkd->bhqd", p, v_cache)
        return (lambda x, *d: x.transpose(*d))(o, 0, 2, 1, 3).reshape(B, Sq, H * Dh) @ wo

    a = _A_ref(A_x, A_k_cache, A_v_cache, A_wq, A_wo)
    b = _B_ref(B_x, B_k_cache, B_v_cache, B_wq, B_wo)
    return jnp.concatenate([a, b], axis=-1)
```

```python
import functools

import jax
import jax.numpy as jnp
from jax import lax
import jax.experimental.pallas as pl
import jax.experimental.pallas.tpu as pltpu

B, SQ, D, H, SK, DH = 16, 32, 1024, 32, 32, 128
HU = 4
UB = H // HU
NU = 2 * UB
NG = NU // 2
W = HU * DH
QS = SQ // 4
MQ = B * QS
BG = 4
R = BG * SQ
LOG2E = 1.4426950408889634

f32, bf16, u32 = jnp.float32, jnp.bfloat16, jnp.uint32

TERMS = {
    (0, 0): ((1, 0), (1, 3), (-1, 4), (1, 6)),
    (0, 1): ((1, 2), (1, 4)),
    (1, 0): ((1, 1), (1, 3)),
    (1, 1): ((1, 0), (-1, 1), (1, 2), (1, 5)),
}

PLAN = dict(
    q_first=dict(outer=(3, 1, 0, 4, 6, 2, 5), inner=(5, 1, 3, 0, 2, 4, 6)),
    q=dict(outer=(1, 3, 2, 4, 0, 5, 6), inner=(5, 1, 3, 0, 2, 4, 6)),
    qa0=dict(outer=(1, 3, 4, 6, 0, 2, 5), inner=(1, 3, 5, 2, 4, 0, 6), qk=(0, 7, 21, 28), pv=(16, 25, 37, 44)),
    qa1=dict(outer=(1, 3, 4, 6, 0, 2, 5), inner=(1, 3, 5, 2, 4, 0, 6), qk=(0, 7, 21, 28), pv=(16, 25, 37, 44)),
    ao0=dict(outer=(1, 3, 4, 6, 0, 2, 5), inner=(1, 5, 3, 2, 4, 0, 6), qk=(3, 7, 21, 28), pv=(16, 25, 37, 44)),
    ao1=dict(outer=(1, 3, 2, 6, 4, 0, 5), inner=(1, 3, 5, 0, 2, 4, 6), qk=(0, 8, 22, 28), pv=(16, 25, 38, 44)),
    ao2=dict(outer=(1, 3, 4, 6, 0, 2, 5), inner=(1, 3, 2, 5, 0, 4, 6), qk=(3, 7, 21, 28), pv=(16, 24, 37, 44)),
    ao3=dict(outer=(1, 3, 2, 6, 4, 0, 5), inner=(1, 3, 4, 2, 5, 0, 6), qk=(0, 7, 22, 28), pv=(16, 25, 37, 47)),
    o0=dict(outer=(1, 3, 2, 4, 0, 5, 6), inner=(5, 1, 3, 0, 2, 4, 6)),
    o1=dict(outer=(1, 3, 4, 6, 0, 2, 5), inner=(5, 1, 3, 0, 2, 4, 6)),
)
RHS_ROWS = 32


def _lhs_operand(i, a):
    return (lambda: a(0, 0) + a(1, 1), lambda: a(1, 0) + a(1, 1), lambda: a(0, 0), lambda: a(1, 1),
            lambda: a(0, 0) + a(0, 1), lambda: a(1, 0) - a(0, 0), lambda: a(0, 1) - a(1, 1))[i]()


def _rhs_operand(i, b):
    return (lambda: b(0, 0) + b(1, 1), lambda: b(0, 0), lambda: b(0, 1) - b(1, 1), lambda: b(1, 0) - b(0, 0),
            lambda: b(1, 1), lambda: b(0, 0) + b(0, 1), lambda: b(1, 0) + b(1, 1))[i]()


def _inner_operands(operand, blk, i):
    outer = {(r, c): operand(i, lambda ro, co: blk(2 * ro + r, 2 * co + c)) for r in range(2) for c in range(2)}
    return [operand(k, lambda r, c: outer[r, c]) for k in range(7)]


def _finished(p, prods, order):
    for quad, terms in TERMS.items():
        if max((t for _, t in terms), key=order.index) == p:
            val = prods[terms[0][1]]
            for sign, t in terms[1:]:
                val = val + prods[t] if sign > 0 else val - prods[t]
            yield quad, val


class _Weights:
    def __init__(self, blk, i, on_demand):
        self.blk, self.i, self.parts = blk, i, None
        if not on_demand:
            self.parts = [_inner_operands(_rhs_operand, lambda r, c: blk(r, c, r0, RHS_ROWS), i)
                          for r0 in range(0, 2 * DH, RHS_ROWS)]

    def get(self, k):
        if self.parts is None:
            outer = lambda r, c: _rhs_operand(self.i, lambda ro, co: self.blk(2 * ro + r, 2 * co + c, 0, 2 * DH))
            return _rhs_operand(k, outer).astype(bf16)
        return jnp.concatenate([part[k] for part in self.parts], axis=0).astype(bf16)


def _strassen2(lhs, blk, done, plan, chain, next_unit=None, cuts=()):
    outer_order, inner_order = plan["outer"], plan["inner"]
    outer = {quad: {} for quad in TERMS}
    result = {quad: {} for quad in TERMS}
    cur = chain.pop() if chain else _Weights(blk, outer_order[0], True)
    for n, i in enumerate(outer_order):
        prods = {}
        for m, k in enumerate(inner_order):
            prods[k] = jnp.dot(lhs(i * 7 + k), cur.get(k), preferred_element_type=f32)
            if m == 0:
                if n < 6:
                    nxt = _Weights(blk, outer_order[n + 1], n + 1 in cuts)
                elif next_unit is not None:
                    chain.append(_Weights(next_unit[0], next_unit[1]["outer"][0], False))
            for quad, val in _finished(k, prods, inner_order):
                outer[quad][i] = val
                for oquad, oval in _finished(i, outer[quad], outer_order):
                    result[oquad][quad] = oval
                    done(oquad, quad, result[oquad])
            yield
        cur = nxt


def _load(view):
    return pltpu.bitcast(view.bitcast(u32)[...], bf16)


def _kernel(a_x, a_k, a_v, a_wq, a_wo, b_x, b_k, b_v, b_wq, b_wo, out_hbm,
            x_buf, xs_a, xs_b, wq_buf, k_buf, v_buf, wo_buf, q_buf, o_even, o_odd, acc, out_buf, sem):
    xs_buf = (xs_a, xs_b)
    o_buf = (o_even, o_odd)

    s_k, s_v, s_wo = NU, NU + NG, NU + 2 * NG
    s_xb, s_out, s_x0, s_w0 = NU + 3 * NG, NU + 3 * NG + 1, NU + 3 * NG + 6, NU + 3 * NG + 10

    def wq_copies(u):
        br, j = divmod(u, UB)
        return [((a_wq, b_wq)[br].at[:, pl.ds(j * W, W)], wq_buf.at[u], sem.at[u])]

    def kv_copies(src, buf, s, g):
        br, j = divmod(g, UB // 2)
        return [(src[br].at[:, pl.ds((2 * j + t) * HU, HU)], buf.at[g, t], sem.at[s + g]) for t in range(2)]

    def wo_copies(g):
        br, j = divmod(g, UB // 2)
        return [((a_wo, b_wo)[br].at[pl.ds(j * 2 * W, 2 * W), pl.ds(h * W, W)], wo_buf.at[g, h], sem.at[s_wo + g])
                for h in range(2)]

    def x0_copy(r, c):
        idx = (slice(None), pl.ds(r * SQ // 2, SQ // 2), pl.ds(c * D // 2, D // 2))
        return a_x.at[idx], x_buf.at[(0,) + idx], sem.at[s_x0 + 2 * r + c]

    def w0_copy(r, c):
        idx = (pl.ds(r * D // 2, D // 2), pl.ds(c * W // 2, W // 2))
        return a_wq.at[idx], wq_buf.at[(0,) + idx], sem.at[s_w0 + 2 * r + c]

    xb_copy = (b_x, x_buf.at[1], sem.at[s_xb])

    def out_copy(n):
        br, h, c0, cols = ((0, 0, 0, W), (0, 1, 0, W), (1, 0, 0, W), (1, 1, 0, W // 2), (1, 1, W // 2, W // 2))[n]
        return pltpu.make_async_copy(out_buf.at[br, h, :, :, pl.ds(c0, cols)],
                                     out_hbm.at[:, :, pl.ds(br * D + h * W + c0, cols)], sem.at[s_out + n])

    def wait(dst, s):
        pltpu.make_async_copy(dst, dst, s).wait()

    def wait_wq(u):
        wait(wq_buf.at[u], sem.at[u])

    def wait_halves(buf, s, g):
        for t in range(2):
            wait(buf.at[g, t], sem.at[s + g])

    copies = [x0_copy(1, 1), x0_copy(1, 0), w0_copy(0, 0), w0_copy(1, 0),
              x0_copy(0, 0), x0_copy(0, 1), w0_copy(1, 1), w0_copy(0, 1)]
    for u in range(1, NU - 2):
        if u == UB // 2:
            copies.append(xb_copy)
        copies += wq_copies(u)
    for g in range(NG + 1):
        if g < NG:
            copies += kv_copies((a_k, b_k), k_buf, s_k, g)
        copies += wo_copies(g - 1) if g else wq_copies(NU - 2) + wq_copies(NU - 1)
        if g < NG:
            copies += kv_copies((a_v, b_v), v_buf, s_v, g)
    for c in copies:
        pltpu.make_async_copy(*c).start()

    @pl.loop(0, 8)
    def _(i):
        acc[i // 4, i // 2 % 2, i % 2] = jnp.zeros(acc.shape[3:], f32)

    def prepare_x(br, outers, b_first=0, b_count=B):
        for b in range(0, b_count, 2):
            row0 = (b_first + b) * QS
            if not isinstance(row0, int):
                row0 = pl.multiple_of(row0, 2 * QS)
            for c in range(2):
                def blk(r, j):
                    both = x_buf[br, pl.ds(b_first + b, 2), r * QS:(r + 1) * QS, 2 * j * DH:2 * (j + 1) * DH]
                    return both.astype(f32).reshape(2 * QS, 2 * DH)[:, c * DH:(c + 1) * DH]
                for i in outers:
                    for k, val in enumerate(_inner_operands(_lhs_operand, blk, i)):
                        xs_buf[br][i * 7 + k, c, pl.ds(row0, 2 * QS)] = val.astype(bf16)

    def wq_block(u):
        def blk(r, c, row0, rows):
            r0 = r * (D // 4) + row0
            both = wq_buf[u, r0:r0 + rows, c // 2 * 2 * DH:(c // 2 + 1) * 2 * DH].astype(f32)
            return both[:, c % 2 * DH:(c % 2 + 1) * DH]
        return blk

    def q_proj(u, br, plan, chain, next_unit=None, cuts=()):
        lhs = lambda p: jnp.concatenate([_load(xs_buf[br].at[p, c]) for c in range(2)], axis=1)

        def done(oquad, quad, blocks):
            c = quad[1]
            if (0, c) in blocks and (1, c) in blocks:
                val = jnp.concatenate([blocks[r, c].reshape(B, QS, DH) for r in range(2)], axis=1)
                q_buf[u, 2 * oquad[1] + c, :, oquad[0]] = val.astype(bf16)
        return _strassen2(lhs, wq_block(u), done, plan, chain, next_unit, cuts)

    lane_batch = lax.broadcasted_iota(jnp.int32, (SK, R), 1) // SQ

    def probabilities(g, t, i):
        rows = pl.ds(i * BG, BG)
        scores = []
        for h in range(HU):
            q = _load(q_buf.at[2 * g + t, h, rows]).reshape(R, DH)
            k = _load(k_buf.at[g, t, rows, h]).reshape(R, DH)
            scores.append(lax.dot_general(k, q, (((1,), (1,)), ((), ())), preferred_element_type=f32))
        probs = []
        for st in scores:
            s = st[3 * SK:]
            for j in (2, 1, 0):
                s = jnp.where(lane_batch == j, st[j * SK:(j + 1) * SK], s)
            e = jnp.exp2((s - jnp.max(s, axis=0, keepdims=True)) * (DH ** -0.5 * LOG2E))
            probs.append(e * (1.0 / jnp.sum(e, axis=0, keepdims=True)))
        return probs

    def weighted_values(g, t, i, probs, parity):
        o = []
        for h in range(HU):
            pt = jnp.concatenate([jnp.where(lane_batch == j, probs[h], 0.0) for j in range(BG)], axis=0)
            v = _load(v_buf.at[g, t, pl.ds(i * BG, BG), h]).reshape(R, DH)
            o.append(lax.dot_general(pt.astype(bf16), v, (((0,), (0,)), ((), ())),
                                     preferred_element_type=f32).reshape(BG, 4, QS, DH))
        for b in range(0, BG, 2):
            row0 = (i * BG + b) * QS
            for j in range(7):
                ops = _inner_operands(_lhs_operand, lambda r, c: o[c][b:b + 2, r].reshape(2 * QS, DH), j)
                for k, val in enumerate(ops):
                    o_buf[parity][j * 7 + k, t, row0:row0 + 2 * QS] = val.astype(bf16)

    def wo_block(g, h):
        def blk(r, c, row0, rows):
            parts = []
            for t in range(2):
                lo, hi = max(row0, t * DH), min(row0 + rows, (t + 1) * DH)
                if lo < hi:
                    r0 = ((HU - 1) * t + r) * DH
                    both = wo_buf[g, h, r0 + lo:r0 + hi, c // 2 * 2 * DH:(c // 2 + 1) * 2 * DH].astype(f32)
                    parts.append(both[:, c % 2 * DH:(c % 2 + 1) * DH])
            return jnp.concatenate(parts, axis=0)
        return blk

    def o_proj(g, h, parity, write_acc, write_out, plan, chain, next_unit=None, cuts=()):
        br = g // (UB // 2)
        lhs = lambda p: jnp.concatenate([_load(o_buf[parity].at[p, t]) for t in range(2)], axis=1)

        def done(oquad, quad, blocks):
            idx = (br, h) + oquad + quad
            blocks[quad] = acc[idx] + blocks[quad]
            if write_acc:
                acc[idx] = blocks[quad]
            r = quad[0]
            if write_out and (r, 0) in blocks and (r, 1) in blocks:
                val = jnp.concatenate([blocks[r, 0], blocks[r, 1]], axis=1).reshape(B, QS, 2 * DH)
                r0, c0 = (2 * oquad[0] + r) * QS, 2 * oquad[1] * DH
                out_buf[br, h, :, r0:r0 + QS, c0:c0 + 2 * DH] = val.astype(bf16)
        return _strassen2(lhs, wo_block(g, h), done, plan, chain, next_unit, cuts)

    def advance(products, count=49):
        for _ in range(count):
            next(products)

    def advance_with_attention(products, plan, g, t, parity):
        probs = {}
        for n in range(50):
            for i in range(B // BG):
                if plan["pv"][i] == n:
                    weighted_values(g, t, i, probs[i], parity)
                if plan["qk"][i] == n:
                    probs[i] = probabilities(g, t, i)
            if n < 49:
                next(products)

    order = PLAN["q_first"]["outer"]
    products = q_proj(0, 0, PLAN["q_first"], [], cuts=(2, 5))
    wait(*x0_copy(1, 1)[1:])
    wait(*x0_copy(1, 0)[1:])
    prepare_x(0, order[:2])
    wait(*w0_copy(0, 0)[1:])
    wait(*w0_copy(1, 0)[1:])
    advance(products, 14)
    wait(*x0_copy(0, 0)[1:])
    wait(*x0_copy(0, 1)[1:])
    prepare_x(0, order[2:])
    wait(*w0_copy(1, 1)[1:])
    advance(products, 21)
    wait(*w0_copy(0, 1)[1:])
    advance(products, 14)

    @pl.loop(1, UB // 2)
    def _(u):
        wait_wq(u)
        advance(q_proj(u, 0, PLAN["q"], []))

    wait(*xb_copy[1:])
    wait_wq(UB // 2)

    @pl.loop(UB // 2, UB)
    def _(u):
        count = B // (UB // 2)
        prepare_x(1, range(7), (u - UB // 2) * count, count)
        advance(q_proj(u, 0, PLAN["q"], []))
        pl.when(u + 1 < UB)(lambda: wait_wq(u + 1))

    @pl.loop(0, 2)
    def _(i):
        u0 = UB + 3 * i
        for j in range(3):
            wait_wq(u0 + j)
        chain = []
        for j in range(3):
            advance(q_proj(u0 + j, 1, PLAN["q"], chain, (wq_block(u0 + j + 1), PLAN["q"]) if j < 2 else None))

    wait_halves(k_buf, s_k, 0)
    wait_wq(NU - 2)
    wait_wq(NU - 1)
    wait_halves(v_buf, s_v, 0)
    chain = []
    for t in range(2):
        plan = PLAN["qa%d" % t]
        products = q_proj(NU - 2 + t, 1, plan, chain, (wq_block(NU - 1), PLAN["qa1"]) if t == 0 else None)
        advance_with_attention(products, plan, 0, t, 0)

    def attend_and_project(g, parity, plans):
        wait_halves(k_buf, s_k, g)
        wait_halves(wo_buf, s_wo, g - 1)
        wait_halves(v_buf, s_v, g)
        chain = []
        for t in range(2):
            products = o_proj(g - 1, t, 1 - parity, True, parity == 0, plans[t], chain,
                              (wo_block(g - 1, 1), plans[1]) if t == 0 else None)
            advance_with_attention(products, plans[t], g, t, parity)

    @pl.loop(0, NG // 2)
    def _(i):
        @pl.when(i == NG // 4)
        def _():
            out_copy(0).start()
            out_copy(1).start()

        attend_and_project(2 * i + 1, 1, (PLAN["ao0"], PLAN["ao1"]))

        @pl.when(i < NG // 2 - 1)
        def _():
            attend_and_project(2 * i + 2, 0, (PLAN["ao2"], PLAN["ao3"]))

        @pl.when(i == NG // 2 - 1)
        def _():
            wait_halves(wo_buf, s_wo, NG - 1)
            advance(o_proj(NG - 1, 0, 1, False, True, PLAN["o0"], []))
            out_copy(2).start()
            products = o_proj(NG - 1, 1, 1, False, True, PLAN["o1"], [], cuts=(5,))
            advance(products, 35)
            out_copy(3).start()
            advance(products, 14)
            out_copy(4).start()

    for n in range(5):
        out_copy(n).wait()


@jax.jit
def pallas_concat_heads__mha_block_cached__mha_block_cached__near_ridge_kernel(
    A_x: jax.Array,
    A_k_cache: jax.Array,
    A_v_cache: jax.Array,
    A_wq: jax.Array,
    A_wo: jax.Array,
    B_x: jax.Array,
    B_k_cache: jax.Array,
    B_v_cache: jax.Array,
    B_wq: jax.Array,
    B_wo: jax.Array,
):
    hbm = pl.BlockSpec(memory_space=pl.ANY)
    factors = pltpu.VMEM((49, 2, MQ, DH), bf16)
    return pl.pallas_call(
        _kernel,
        out_shape=jax.ShapeDtypeStruct((B, SQ, 2 * D), bf16),
        in_specs=[hbm] * 10,
        out_specs=hbm,
        scratch_shapes=[
            pltpu.VMEM((2, B, SQ, D), bf16),
            factors, factors,
            pltpu.VMEM((NU, D, W), bf16),
            pltpu.VMEM((NG, 2, B, HU, SK, DH), bf16),
            pltpu.VMEM((NG, 2, B, HU, SK, DH), bf16),
            pltpu.VMEM((NG, 2, 2 * W, W), bf16),
            pltpu.VMEM((NU, HU, B, 2, 2 * QS, DH), bf16),
            factors, factors,
            pltpu.VMEM((2, 2, 2, 2, 2, 2, MQ, DH), f32),
            pltpu.VMEM((2, 2, B, SQ, W), bf16),
            pltpu.SemaphoreType.DMA((NU + 3 * NG + 14,)),
        ],
        compiler_params=pltpu.CompilerParams(
            vmem_limit_bytes=100 * 2**20,
            disable_bounds_checks=True,
            disable_semaphore_checks=True,
        ),
    )(A_x, A_k_cache, A_v_cache, A_wq, A_wo, B_x, B_k_cache, B_v_cache, B_wq, B_wo)
```

```python
import jax
import jax.numpy as jnp
from jax import lax
import jax.experimental.pallas as pl
import jax.experimental.pallas.tpu as pltpu

B, SQ, D, H, SK, DH = 16, 32, 1024, 32, 32, 128
HU = 4
UB = H // HU
NU = 2 * UB
NG = NU // 2
W = HU * DH
QS = SQ // 4
MQ = B * QS
BG = 4
R = BG * SQ
NUM_SEMS = NU + 2 * NG + 10
LOG2E = 1.4426950408889634

f32, bf16 = jnp.float32, jnp.bfloat16

TERMS = {
    (0, 0): ((1, 0), (1, 3), (-1, 4), (1, 6)),
    (0, 1): ((1, 2), (1, 4)),
    (1, 0): ((1, 1), (1, 3)),
    (1, 1): ((1, 0), (-1, 1), (1, 2), (1, 5)),
}

PLAN = dict(
    q_first=dict(outer=(1, 3, 4, 0, 6, 2, 5), inner=(1, 0, 3, 5, 2, 6, 4)),
    q=dict(outer=(1, 3, 2, 4, 0, 6, 5), inner=(1, 5, 3, 2, 0, 6, 4)),
    qx=dict(outer=(4, 3, 2, 0, 1, 5, 6), inner=(1, 3, 0, 6, 2, 5, 4)),
    qb0=dict(outer=(1, 3, 2, 4, 0, 5, 6), inner=(1, 3, 5, 0, 2, 6, 4)),
    qb1=dict(outer=(0, 1, 4, 3, 2, 5, 6), inner=(1, 0, 4, 3, 6, 2, 5)),
    qb2=dict(outer=(3, 4, 2, 1, 0, 5, 6), inner=(3, 1, 4, 0, 2, 6, 5)),
    qc=dict(outer=(1, 3, 2, 4, 0, 5, 6), inner=(1, 3, 5, 2, 0, 6, 4)),
    qa0=dict(outer=(3, 4, 0, 6, 1, 2, 5), inner=(1, 3, 0, 2, 4, 5, 6), qk=(3, 7, 21, 35), pv=(16, 30, 37, 44)),
    qa1=dict(outer=(1, 3, 4, 6, 2, 0, 5), inner=(1, 3, 0, 2, 5, 4, 6), qk=(0, 8, 23, 28), pv=(16, 26, 37, 47)),
    ao0=dict(outer=(1, 3, 4, 6, 0, 5, 2), inner=(1, 0, 3, 5, 2, 4, 6), qk=(3, 7, 27, 28), pv=(16, 23, 37, 43)),
    ao1=dict(outer=(4, 2, 1, 3, 0, 5, 6), inner=(1, 5, 3, 0, 6, 4, 2), qk=(0, 8, 22, 28), pv=(16, 24, 38, 46)),
    ao2=dict(outer=(1, 3, 2, 4, 0, 5, 6), inner=(1, 3, 5, 0, 2, 4, 6), qk=(3, 7, 20, 30), pv=(16, 24, 37, 44)),
    ao3=dict(outer=(1, 3, 4, 6, 2, 0, 5), inner=(1, 3, 4, 2, 5, 0, 6), qk=(1, 8, 21, 28), pv=(16, 25, 37, 44)),
    ao4=dict(outer=(1, 3, 4, 6, 0, 5, 2), inner=(1, 0, 3, 5, 2, 4, 6), qk=(3, 7, 27, 28), pv=(16, 23, 37, 43)),
    ao5=dict(outer=(4, 2, 3, 0, 1, 5, 6), inner=(1, 5, 3, 6, 0, 4, 2), qk=(0, 8, 22, 28), pv=(16, 24, 38, 44)),
    o0=dict(outer=(1, 3, 2, 4, 0, 5, 6), inner=(5, 2, 1, 0, 4, 3, 6)),
    o1=dict(outer=(3, 4, 0, 6, 2, 1, 5), inner=(0, 1, 3, 5, 2, 4, 6)),
)
RHS_ROWS = 16


def _lhs_operand(i, a):
    return (lambda: a(0, 0) + a(1, 1), lambda: a(1, 0) + a(1, 1), lambda: a(0, 0), lambda: a(1, 1),
            lambda: a(0, 0) + a(0, 1), lambda: a(1, 0) - a(0, 0), lambda: a(0, 1) - a(1, 1))[i]()


def _rhs_operand(i, b):
    return (lambda: b(0, 0) + b(1, 1), lambda: b(0, 0), lambda: b(0, 1) - b(1, 1), lambda: b(1, 0) - b(0, 0),
            lambda: b(1, 1), lambda: b(0, 0) + b(0, 1), lambda: b(1, 0) + b(1, 1))[i]()


def _inner_operands(operand, blk, i):
    outer = {(r, c): operand(i, lambda ro, co: blk(2 * ro + r, 2 * co + c)) for r in range(2) for c in range(2)}
    return [operand(k, lambda r, c: outer[r, c]) for k in range(7)]


def _finished(p, prods, order):
    for quad, terms in TERMS.items():
        if max((t for _, t in terms), key=order.index) == p:
            val = prods[terms[0][1]]
            for sign, t in terms[1:]:
                val = val + prods[t] if sign > 0 else val - prods[t]
            yield quad, val


class _Weights:
    def __init__(self, blk, i, on_demand):
        self.blk, self.i, self.parts = blk, i, None
        if not on_demand:
            self.parts = [_inner_operands(_rhs_operand, lambda r, c: blk(r, c, r0, RHS_ROWS), i)
                          for r0 in range(0, 2 * DH, RHS_ROWS)]

    def get(self, k):
        if self.parts is None:
            outer = lambda r, c: _rhs_operand(self.i, lambda ro, co: self.blk(2 * ro + r, 2 * co + c, 0, 2 * DH))
            return _rhs_operand(k, outer).astype(bf16)
        return jnp.concatenate([part[k] for part in self.parts], axis=0).astype(bf16)


def _strassen2(lhs, blk, done, plan, chain, next_unit=None, cuts=()):
    outer_order, inner_order = plan["outer"], plan["inner"]
    outer = {quad: {} for quad in TERMS}
    result = {quad: {} for quad in TERMS}
    cur = chain.pop() if chain else _Weights(blk, outer_order[0], True)
    for n, i in enumerate(outer_order):
        prods = {}
        for m, k in enumerate(inner_order):
            prods[k] = jnp.dot(lhs(i * 7 + k), cur.get(k), preferred_element_type=f32)
            if m == 0:
                if n < 6:
                    nxt = _Weights(blk, outer_order[n + 1], n + 1 in cuts)
                elif next_unit is not None:
                    chain.append(_Weights(next_unit[0], next_unit[1]["outer"][0], False))
            for quad, val in _finished(k, prods, inner_order):
                outer[quad][i] = val
                for oquad, oval in _finished(i, outer[quad], outer_order):
                    result[oquad][quad] = oval
                    done(oquad, quad, result[oquad])
            yield
        cur = nxt


def _kernel(a_x, a_k, a_v, a_wq, a_wo, b_x, b_k, b_v, b_wq, b_wo, out_hbm,
            x_buf, xs_a, xs_b, wq_buf, kv_buf, wo_buf, q_buf, o_even, o_odd, acc, out_buf, sem):
    xs_buf = (xs_a, xs_b)
    o_buf = (o_even, o_odd)

    s_kv, s_wo, s_x0, s_w0, s_xb, s_out = NU, NU + NG, NU + 2 * NG, NU + 2 * NG + 4, NU + 2 * NG + 8, NU + 2 * NG + 9
    assert s_out + 1 == NUM_SEMS

    def wq_copies(u0, count=1):
        return [((a_wq, b_wq)[u // UB].at[:, pl.ds(u % UB * W, W)], wq_buf.at[u], sem.at[u0])
                for u in range(u0, u0 + count)]

    def kv_copies(src, which, g):
        br, j = divmod(g, UB // 2)
        return [(src[br].at[:, pl.ds((2 * j + t) * HU, HU)], kv_buf.at[g, which, t], sem.at[s_kv + g])
                for t in range(2)]

    def wo_copies(g):
        br, j = divmod(g, UB // 2)
        return [((a_wo, b_wo)[br].at[pl.ds(j * 2 * W, 2 * W), pl.ds(h * W, W)], wo_buf.at[g, h], sem.at[s_wo + g])
                for h in range(2)]

    def x0_copy(r, c):
        idx = (slice(None), pl.ds(r * SQ // 2, SQ // 2), pl.ds(c * D // 2, D // 2))
        return a_x.at[idx], x_buf.at[(0,) + idx], sem.at[s_x0 + 2 * r + c]

    def w0_copy(r, c):
        idx = (pl.ds(r * D // 2, D // 2), pl.ds(c * W // 2, W // 2))
        return a_wq.at[idx], wq_buf.at[(0,) + idx], sem.at[s_w0 + 2 * r + c]

    xb_copy = (b_x, x_buf.at[1], sem.at[s_xb])

    def start_out(br, h, r0=0, rows=SQ, c0=0, cols=W):
        pltpu.make_async_copy(out_buf.at[br, h, :, pl.ds(r0, rows), pl.ds(c0, cols)],
                              out_hbm.at[:, pl.ds(r0, rows), pl.ds(br * D + h * W + c0, cols)],
                              sem.at[s_out]).start()

    def wait(dst, s):
        pltpu.make_async_copy(dst, dst, s).wait()

    def wait_wq(u0, count=1):
        wait(wq_buf.at[pl.ds(u0, count)], sem.at[u0])

    copies = [x0_copy(1, 1), x0_copy(1, 0), w0_copy(0, 0), w0_copy(1, 0),
              x0_copy(0, 0), x0_copy(0, 1), w0_copy(1, 1), w0_copy(0, 1)]
    for u in range(1, UB - 1):
        if u == 3:
            copies.append(xb_copy)
        copies += wq_copies(u)
    copies += wq_copies(UB, 3) + wq_copies(UB + 3, 3) + wq_copies(UB - 1) + wq_copies(NU - 2, 2)
    for g in range(NG):
        copies += kv_copies((a_k, b_k), 0, g) + kv_copies((a_v, b_v), 1, g) + wo_copies(g)
    for c in copies:
        pltpu.make_async_copy(*c).start()

    @pl.loop(0, 8)
    def _(i):
        acc[i // 4, i // 2 % 2, i % 2] = jnp.zeros(acc.shape[3:], f32)

    def prepare_x(br, outers, b_first=0, b_count=B):
        for b in range(0, b_count, 2):
            row0 = (b_first + b) * QS
            if not isinstance(row0, int):
                row0 = pl.multiple_of(row0, 2 * QS)
            for c in range(2):
                def blk(r, j):
                    both = x_buf[br, pl.ds(b_first + b, 2), r * QS:(r + 1) * QS, 2 * j * DH:2 * (j + 1) * DH]
                    return both.astype(f32).reshape(2 * QS, 2 * DH)[:, c * DH:(c + 1) * DH]
                for i in outers:
                    for k, val in enumerate(_inner_operands(_lhs_operand, blk, i)):
                        xs_buf[br][i * 7 + k, c, pl.ds(row0, 2 * QS)] = val.astype(bf16)
                    yield

    def wq_block(u):
        def blk(r, c, row0, rows):
            r0 = r * (D // 4) + row0
            both = wq_buf[u, r0:r0 + rows, c // 2 * 2 * DH:(c // 2 + 1) * 2 * DH].astype(f32)
            return both[:, c % 2 * DH:(c % 2 + 1) * DH]
        return blk

    def q_proj(u, br, plan, chain, next_unit=None, cuts=()):
        lhs = lambda p: jnp.concatenate([xs_buf[br][p, c] for c in range(2)], axis=1)

        def done(oquad, quad, blocks):
            c = quad[1]
            if (0, c) in blocks and (1, c) in blocks:
                val = jnp.concatenate([blocks[r, c].reshape(B, QS, DH) for r in range(2)], axis=1)
                q_buf[u, 2 * oquad[1] + c, :, oquad[0]] = val.astype(bf16)
        return _strassen2(lhs, wq_block(u), done, plan, chain, next_unit, cuts)

    lane_batch = lax.broadcasted_iota(jnp.int32, (SK, R), 1) // SQ

    def probabilities(g, t, i):
        rows = pl.ds(i * BG, BG)
        scores = []
        for h in range(HU):
            q = q_buf[2 * g + t, h, rows].reshape(R, DH)
            k = kv_buf[g, 0, t, rows, h].reshape(R, DH)
            scores.append(lax.dot_general(k, q, (((1,), (1,)), ((), ())), preferred_element_type=f32))
        probs = []
        for st in scores:
            s = st[3 * SK:]
            for j in (2, 1, 0):
                s = jnp.where(lane_batch == j, st[j * SK:(j + 1) * SK], s)
            e = jnp.exp2((s - jnp.max(s, axis=0, keepdims=True)) * (DH ** -0.5 * LOG2E))
            probs.append(e / jnp.sum(e, axis=0, keepdims=True))
        return probs

    def weighted_values(g, t, i, probs, parity):
        o = []
        for h in range(HU):
            pt = jnp.concatenate([jnp.where(lane_batch == j, probs[h], 0.0) for j in range(BG)], axis=0)
            v = kv_buf[g, 1, t, pl.ds(i * BG, BG), h].reshape(R, DH)
            o.append(lax.dot_general(pt.astype(bf16), v, (((0,), (0,)), ((), ())),
                                     preferred_element_type=f32).reshape(BG, 4, QS, DH))
        for b in range(0, BG, 2):
            row0 = (i * BG + b) * QS
            for j in range(7):
                ops = _inner_operands(_lhs_operand, lambda r, c: o[c][b:b + 2, r].reshape(2 * QS, DH), j)
                for k, val in enumerate(ops):
                    o_buf[parity][j * 7 + k, t, row0:row0 + 2 * QS] = val.astype(bf16)

    def wo_block(g, h):
        def blk(r, c, row0, rows):
            parts = []
            for t in range(2):
                lo, hi = max(row0, t * DH), min(row0 + rows, (t + 1) * DH)
                if lo < hi:
                    r0 = ((HU - 1) * t + r) * DH
                    both = wo_buf[g, h, r0 + lo:r0 + hi, c // 2 * 2 * DH:(c // 2 + 1) * 2 * DH].astype(f32)
                    parts.append(both[:, c % 2 * DH:(c % 2 + 1) * DH])
            return jnp.concatenate(parts, axis=0)
        return blk

    def o_proj(g, h, parity, write_acc, write_out, plan, chain, next_unit=None, send=False):
        br = g // (UB // 2)
        lhs = lambda p: jnp.concatenate([o_buf[parity][p, t] for t in range(2)], axis=1)

        def done(oquad, quad, blocks):
            idx = (br, h) + oquad + quad
            blocks[quad] = acc[idx] + blocks[quad]
            if write_acc:
                acc[idx] = blocks[quad]
            r = quad[0]
            if write_out and (r, 0) in blocks and (r, 1) in blocks:
                val = jnp.concatenate([blocks[r, 0], blocks[r, 1]], axis=1).reshape(B, QS, 2 * DH)
                r0, c0 = (2 * oquad[0] + r) * QS, 2 * oquad[1] * DH
                out_buf[br, h, :, r0:r0 + QS, c0:c0 + 2 * DH] = val.astype(bf16)
                if send:
                    start_out(br, h, r0, QS, c0, 2 * DH)
        return _strassen2(lhs, wo_block(g, h), done, plan, chain, next_unit)

    def advance(products, count=49):
        for _ in range(count):
            next(products)

    def advance_with_attention(products, plan, g, t, parity):
        probs = {}
        for n in range(50):
            for i in range(B // BG):
                if plan["pv"][i] == n:
                    weighted_values(g, t, i, probs[i], parity)
                if plan["qk"][i] == n:
                    probs[i] = probabilities(g, t, i)
            if n < 49:
                next(products)

    def project_queries():
        order = PLAN["q_first"]["outer"]
        products = q_proj(0, 0, PLAN["q_first"], [], cuts=(2, 5))
        wait(*x0_copy(1, 1)[1:])
        wait(*x0_copy(1, 0)[1:])
        list(prepare_x(0, order[:2]))
        wait(*w0_copy(0, 0)[1:])
        wait(*w0_copy(1, 0)[1:])
        advance(products, 14)
        wait(*x0_copy(0, 0)[1:])
        wait(*x0_copy(0, 1)[1:])
        list(prepare_x(0, order[2:]))
        wait(*w0_copy(1, 1)[1:])
        advance(products, 21)
        wait(*w0_copy(0, 1)[1:])
        advance(products, 14)

        @pl.loop(1, 3)
        def _(u):
            wait_wq(u)
            advance(q_proj(u, 0, PLAN["q"], []))

        wait(*xb_copy[1:])
        wait_wq(3)

        @pl.loop(3, UB - 1)
        def _(u):
            factors = prepare_x(1, range(7), (u - 3) * (B // 4), B // 4)
            for n, _ in enumerate(q_proj(u, 0, PLAN["qx"], [])):
                if n % 5 < 3:
                    next(factors, None)
            assert next(factors, "done") == "done"
            pl.when(u < UB - 2)(lambda: wait_wq(u + 1))

        @pl.loop(0, 2)
        def _(i):
            u0 = UB + 3 * i
            wait_wq(u0, 3)
            chain = []
            for j in range(3):
                advance(q_proj(u0 + j, 1, PLAN["qb%d" % j], chain,
                               (wq_block(u0 + j + 1), PLAN["qb%d" % (j + 1)]) if j < 2 else None))

        wait_wq(UB - 1)
        wait_wq(NU - 2, 2)
        wait(kv_buf.at[0], sem.at[s_kv])
        chain = []
        advance(q_proj(UB - 1, 0, PLAN["qc"], chain, (wq_block(NU - 2), PLAN["qa0"])))
        for t in range(2):
            plan = PLAN["qa%d" % t]
            products = q_proj(NU - 2 + t, 1, plan, chain, (wq_block(NU - 1), PLAN["qa1"]) if t == 0 else None)
            advance_with_attention(products, plan, 0, t, 0)

    def attend_and_project(g, parity, plans, next_unit=None):
        wait(wo_buf.at[g - 1], sem.at[s_wo + g - 1])
        wait(kv_buf.at[g], sem.at[s_kv + g])
        chain = []
        for t in range(2):
            products = o_proj(g - 1, t, 1 - parity, True, parity == 0, plans[t], chain,
                              (wo_block(g - 1, 1), plans[1]) if t == 0 else next_unit)
            advance_with_attention(products, plans[t], g, t, parity)
        return chain

    @pl.loop(0, NG // 2 + 1)
    def _(i):
        pl.when(i == 0)(project_queries)

        @pl.when(jnp.logical_and(i > 0, i < NG // 2))
        def _():
            attend_and_project(2 * i - 1, 1, (PLAN["ao0"], PLAN["ao1"]))
            attend_and_project(2 * i, 0, (PLAN["ao2"], PLAN["ao3"]))

        @pl.when(i == NG // 2)
        def _():
            start_out(0, 0)
            start_out(0, 1)
            wait(wo_buf.at[NG - 1], sem.at[s_wo + NG - 1])
            chain = attend_and_project(NG - 1, 1, (PLAN["ao4"], PLAN["ao5"]), (wo_block(NG - 1, 0), PLAN["o0"]))
            advance(o_proj(NG - 1, 0, 1, False, True, PLAN["o0"], chain, (wo_block(NG - 1, 1), PLAN["o1"])))
            start_out(1, 0)
            advance(o_proj(NG - 1, 1, 1, False, True, PLAN["o1"], chain, send=True))

    wait(out_buf, sem.at[s_out])


@jax.jit
def pallas_concat_heads__mha_block_cached__mha_block_cached__near_ridge_kernel(
    A_x: jax.Array,
    A_k_cache: jax.Array,
    A_v_cache: jax.Array,
    A_wq: jax.Array,
    A_wo: jax.Array,
    B_x: jax.Array,
    B_k_cache: jax.Array,
    B_v_cache: jax.Array,
    B_wq: jax.Array,
    B_wo: jax.Array,
):
    hbm = pl.BlockSpec(memory_space=pl.ANY)
    factors = pltpu.VMEM((49, 2, MQ, DH), bf16)
    return pl.pallas_call(
        _kernel,
        out_shape=jax.ShapeDtypeStruct((B, SQ, 2 * D), bf16),
        in_specs=[hbm] * 10,
        out_specs=hbm,
        scratch_shapes=[
            pltpu.VMEM((2, B, SQ, D), bf16),
            factors, factors,
            pltpu.VMEM((NU, D, W), bf16),
            pltpu.VMEM((NG, 2, 2, B, HU, SK, DH), bf16),
            pltpu.VMEM((NG, 2, 2 * W, W), bf16),
            pltpu.VMEM((NU, HU, B, 2, 2 * QS, DH), bf16),
            factors, factors,
            pltpu.VMEM((2, 2, 2, 2, 2, 2, MQ, DH), f32),
            pltpu.VMEM((2, 2, B, SQ, W), bf16),
            pltpu.SemaphoreType.DMA((NUM_SEMS,)),
        ],
        compiler_params=pltpu.CompilerParams(
            vmem_limit_bytes=100 * 2**20,
            disable_bounds_checks=True,
            disable_semaphore_checks=True,
        ),
    )(A_x, A_k_cache, A_v_cache, A_wq, A_wo, B_x, B_k_cache, B_v_cache, B_wq, B_wo)
```
